```python
import jax
import jax.numpy as jnp

def _softmax(x, axis=-1):
    return jax.nn.softmax(x, axis=axis)

def _gelu(x):
    return jax.nn.gelu(x, approximate=True)

def _silu(x):
    return jax.nn.silu(x)

def _sigmoid(x):
    return jax.nn.sigmoid(x)

def _layernorm(x, axis=-1, eps=1e-05):
    m = jnp.mean(x, axis=axis, keepdims=True)
    v = jnp.var(x, axis=axis, keepdims=True)
    return (x - m) / jnp.sqrt(v + eps)

def _scatter_add(tgt, idx, src, axis=0):
    return tgt.at[idx].add(src)

def _segment_sum(src, seg, n):
    return jax.ops.segment_sum(src, seg, n)

class _Rng:

    def __init__(self, key):
        self._k = key

    def _next(self):
        self._k, sub = jax.random.split(self._k)
        return sub

    def normal(self, shape):
        return jax.random.normal(self._next(), shape, dtype=jnp.bfloat16)

    def randint(self, lo, hi, shape):
        return jax.random.randint(self._next(), shape, lo, hi, dtype=jnp.int32)

    def uniform(self, shape, lo=0.0, hi=1.0):
        return jax.random.uniform(self._next(), shape, jnp.bfloat16, lo, hi)

    def permutation(self, n):
        return jax.random.permutation(self._next(), n)
kernel_name = 'adaLN_cond__sliding_block_cached__dense_activation_gelu__decode'

def setup_inputs():
    _rng = _Rng(jax.random.key(int.from_bytes(__import__("os").urandom(4), "little")))
    _w = lambda a: (lambda t: t.astype(jnp.bfloat16) if jnp.issubdtype(t.dtype, jnp.floating) else t)(jnp.asarray(a))

    def _A_setup():
        B, Sq, D = (4, 1, 640)
        Hq, Hkv, Sk, Dh = (32, 32, 8192, 128)
        assert Hq % Hkv == 0, (Hq, Hkv)
        return {'x': _w((lambda *s: _rng.normal(s) * 0.05)(B, Sq, D)), 'k_cache': _w((lambda *s: _rng.normal(s) * 0.05)(B, Hkv, Sk, Dh)), 'v_cache': _w((lambda *s: _rng.normal(s) * 0.05)(B, Hkv, Sk, Dh)), 'wq': _w((lambda *s: _rng.normal(s) * 0.05)(D, Hq * Dh) * D ** (-0.5)), 'wo': _w((lambda *s: _rng.normal(s) * 0.05)(Hq * Dh, D) * (Hq * Dh) ** (-0.5))}
    _A_in = _A_setup()

    def _B_setup():
        B, S, D, F = (4, 1, 640, 1728)
        return {'x': _w((lambda *s: _rng.normal(s) * 0.05)(B, S, D)), 'w1': _w((lambda *s: _rng.normal(s) * 0.05)(D, F) * D ** (-0.5)), 'b1': _w((lambda *s: _rng.normal(s) * 0.05)(F) * 0.01), 'w2': _w((lambda *s: _rng.normal(s) * 0.05)(F, D) * F ** (-0.5)), 'b2': _w((lambda *s: _rng.normal(s) * 0.05)(D) * 0.01)}
    _B_in = _B_setup()
    return {'A_x': _A_in['x'], 'A_k_cache': _A_in['k_cache'], 'A_v_cache': _A_in['v_cache'], 'A_wq': _A_in['wq'], 'A_wo': _A_in['wo'], 'B_x': _B_in['x'], 'B_w1': _B_in['w1'], 'B_b1': _B_in['b1'], 'B_w2': _B_in['w2'], 'B_b2': _B_in['b2'], 'c': _w((lambda *s: _rng.normal(s) * 0.05)(4, 640)), 'w_mod': _w((lambda *s: _rng.normal(s) * 0.05)(640, 6 * 640) * 640 ** (-0.5))}

def reference(A_x, A_k_cache, A_v_cache, A_wq, A_wo, B_x, B_w1, B_b1, B_w2, B_b2, c, w_mod):

    def _A_ref(x, k_cache, v_cache, wq, wo):
        B, Sq, D = x.shape
        Hq, Dh = (32, 128)
        Hkv, Sk = (k_cache.shape[1], k_cache.shape[2])
        W = min(4096, max(256, Sk // 4))
        rep = Hq // Hkv
        q = (lambda x, *d: x.transpose(*d))((x @ wq).reshape(B, Sq, Hq, Dh), 0, 2, 1, 3)
        k = jnp.repeat(k_cache[:, :, Sk - W:, :], rep, axis=1)
        v = jnp.repeat(v_cache[:, :, Sk - W:, :], rep, axis=1)
        scores = jnp.einsum('bhqd,bhkd->bhqk', q, k) * Dh ** (-0.5)
        p = _softmax(scores, axis=-1)
        o = jnp.einsum('bhqk,bhkd->bhqd', p, v)
        return (lambda x, *d: x.transpose(*d))(o, 0, 2, 1, 3).reshape(B, Sq, Hq * Dh) @ wo

    def _B_ref(x, w1, b1, w2, b2):
        h = jnp.einsum('bsd,df->bsf', x, w1) + b1
        h = _gelu(h)
        return jnp.einsum('bsf,fd->bsd', h, w2) + b2
    x = A_x
    mod = (_silu(c) @ w_mod).reshape(c.shape[0], 6, 1, -1)
    sa, ca, ga, sb, cb, gb = (mod[:, 0].copy(), mod[:, 1].copy(), mod[:, 2].copy(), mod[:, 3].copy(), mod[:, 4].copy(), mod[:, 5].copy())
    h = _layernorm(x, axis=-1) * (1 + ca) + sa
    x = x + ga * _A_ref(h, A_k_cache, A_v_cache, A_wq, A_wo)
    h = _layernorm(x, axis=-1) * (1 + cb) + sb
    x = x + gb * _B_ref(h, B_w1, B_b1, B_w2, B_b2)
    return x
```

```python
import jax
import jax.numpy as jnp
from jax import lax
import jax.experimental.pallas as pl
import jax.experimental.pallas.tpu as pltpu

_BF16 = jnp.bfloat16
_F32 = jnp.float32
_HQ, _DH = 32, 128
_KV_ROWS = 128
_W_ROWS = 32
_LOOKAHEAD = 3


def _layernorm(x, eps=1e-5):
    m = jnp.mean(x, axis=-1, keepdims=True)
    d = x - m
    v = jnp.mean(d * d, axis=-1, keepdims=True)
    return d * lax.rsqrt(v + eps)


def _dot(a, b):
    return jnp.dot(a, b, preferred_element_type=_F32)


def _dot_nt(a, b):
    return lax.dot_general(a, b, (((1,), (1,)), ((), ())), preferred_element_type=_F32)


def _wait_filled(ref, sem):
    pltpu.make_async_copy(ref, ref, sem).wait()


@jax.jit
def pallas_adaLN_cond__sliding_block_cached__dense_activation_gelu__decode_kernel(
    A_x: jax.Array,
    A_k_cache: jax.Array,
    A_v_cache: jax.Array,
    A_wq: jax.Array,
    A_wo: jax.Array,
    B_x: jax.Array,
    B_w1: jax.Array,
    B_b1: jax.Array,
    B_w2: jax.Array,
    B_b2: jax.Array,
    c: jax.Array,
    w_mod: jax.Array,
):
    del B_x
    B, Sq, D = A_x.shape
    Hkv, Sk = A_k_cache.shape[1], A_k_cache.shape[2]
    F = B_w1.shape[1]
    assert Sq == 1 and Hkv == _HQ
    W = min(4096, max(256, Sk // 4))
    S0 = Sk - W
    H = _HQ
    n_units = H * B
    n_slots = 2 * B
    assert _LOOKAHEAD < B
    QC = 1024
    n_qc = H * _DH // QC
    f_chunks = [(0, 640), (640, 576), (1216, 512)]
    assert sum(n for _, n in f_chunks) == F

    def kernel(
        x_hbm, k_hbm, v_hbm, wq_hbm, wo_hbm, w1t_hbm, b1_hbm, w2_hbm, b2_hbm, c_hbm, wm_hbm,
        o_ref,
        x_v, c_v, b1_v, b2_v, wm_v, wq_v, wo_v, w1t_v, w2_v, k_v, v_v, q_v,
        s_small, s_wm, s_wq, s_wo, s_w1, s_w2, s_k, s_v,
    ):
        def start_cols(src, dst, col0, ncols, sem):
            def body(i, _):
                for p in range(2):
                    r = pl.ds(pl.multiple_of((2 * i + p) * 16, 16), 16)
                    pltpu.make_async_copy(
                        src.at[r, pl.ds(col0, ncols)], dst.at[r, pl.ds(col0, ncols)], sem
                    ).start(priority=p)
            lax.fori_loop(0, D // 32, body, None)

        def start_rows(src, dst, row0, nrows, sem):
            def body(i, _):
                for p in range(2):
                    r = pl.ds(pl.multiple_of(row0 + (2 * i + p) * _W_ROWS, _W_ROWS), _W_ROWS)
                    pltpu.make_async_copy(src.at[r], dst.at[r], sem).start(priority=p)
            lax.fori_loop(0, nrows // (2 * _W_ROWS), body, None)

        def kv_copy(src, dst, sem, h, b, t):
            slot = (h % 2) * B + b
            return pltpu.make_async_copy(
                src.at[b, h, pl.ds(S0 + t * _KV_ROWS, _KV_ROWS)],
                dst.at[slot, pl.ds(t * _KV_ROWS, _KV_ROWS)],
                sem.at[slot],
            )

        def start_unit(hk, hv, b):
            for t in range(W // _KV_ROWS):
                both = hk is not None and hv is not None
                if hk is not None:
                    kv_copy(k_hbm, k_v, s_k, hk, b, t).start(priority=0 if both else t % 2)
                if hv is not None:
                    kv_copy(v_hbm, v_v, s_v, hv, b, t).start(priority=1 if both else t % 2)

        def start_step_unit(i, b):
            i, b = i + b // B, b % B
            start_unit(i, i - 1, b)

        def wait_cols(dst, col0, ncols, sem):
            _wait_filled(dst.at[:, pl.ds(col0, ncols)], sem)

        def scores(h, b, s):
            slot = (h % 2) * B + b
            _wait_filled(k_v.at[slot], s_k.at[slot])
            sb = _dot_nt(q_v[h], k_v[slot])
            return sb if s is None else jnp.where(lax.broadcasted_iota(jnp.int32, sb.shape, 0) == b, sb, s)

        def values(h, b, p, o):
            slot = (h % 2) * B + b
            _wait_filled(v_v.at[slot], s_v.at[slot])
            ob = _dot(p, v_v[slot])
            return ob if o is None else jnp.where(lax.broadcasted_iota(jnp.int32, ob.shape, 0) == b, ob, o)

        def softmax_parts(s):
            s = s * (_DH ** -0.5)
            e = jnp.exp(s - jnp.max(s, axis=-1, keepdims=True))
            return e.astype(_BF16), jnp.sum(e, axis=-1, keepdims=True)

        def out_proj(h, o, l):
            r = pl.ds(pl.multiple_of(h * _DH, _DH), _DH)
            return _dot((o / l).astype(_BF16), wo_v[r, :])

        small = [
            pltpu.make_async_copy(src, dst, s_small.at[j])
            for j, (src, dst) in enumerate(
                ((c_hbm, c_v), (x_hbm, x_v), (b1_hbm, b1_v), (b2_hbm, b2_v))
            )
        ]
        for cp in small:
            cp.start()
        start_cols(wm_hbm, wm_v, 0, 2 * D, s_wm.at[0])
        start_cols(wq_hbm, wq_v, 0, QC, s_wq.at[0])
        start_cols(wq_hbm, wq_v, QC, QC, s_wq.at[1])
        for cp in small:
            cp.wait()
        cf = c_v[...].astype(_F32)
        sc = (cf * jax.nn.sigmoid(cf)).astype(_BF16)
        x = x_v[...].astype(_F32)
        wait_cols(wm_v, 0, 2 * D, s_wm.at[0])
        mod_a = _dot(sc, wm_v[:, 0:2 * D])
        h1 = (_layernorm(x) * (1.0 + mod_a[:, D:]) + mod_a[:, :D]).astype(_BF16)

        def q_chunk(j):
            wait_cols(wq_v, j * QC, QC, s_wq.at[j])
            q = _dot(h1, wq_v[:, j * QC:(j + 1) * QC]).astype(_BF16)
            for t in range(QC // _DH):
                q_v[j * (QC // _DH) + t] = q[:, t * _DH:(t + 1) * _DH]

        start_cols(wq_hbm, wq_v, 2 * QC, QC, s_wq.at[2])
        q_chunk(0)
        start_cols(wq_hbm, wq_v, 3 * QC, QC, s_wq.at[3])
        q_chunk(1)
        start_cols(wm_hbm, wm_v, 2 * D, 2 * D, s_wm.at[1])
        q_chunk(2)
        start_cols(wm_hbm, wm_v, 4 * D, 2 * D, s_wm.at[2])
        q_chunk(3)
        start_rows(wo_hbm, wo_v, 0, 1024, s_wo)
        wait_cols(wm_v, 2 * D, 2 * D, s_wm.at[1])
        mod_b = _dot(sc, wm_v[:, 2 * D:4 * D])
        start_rows(wo_hbm, wo_v, 1024, 1024, s_wo)
        wait_cols(wm_v, 4 * D, 2 * D, s_wm.at[2])
        mod_c = _dot(sc, wm_v[:, 4 * D:6 * D])
        start_rows(wo_hbm, wo_v, 2048, 2048, s_wo)

        for b in range(B):
            start_unit(0, None, b)
        s = None
        for b in range(B):
            if b >= B - _LOOKAHEAD - 1 + 1:
                start_unit(1, 0, b - (B - _LOOKAHEAD))
            s = scores(0, b, s)
        p, l = softmax_parts(s)
        _wait_filled(wo_v, s_wo)

        def step(i, carry, start):
            p, l, acc = carry
            s = o = None
            for b in range(B):
                start(i, b)
                s = scores(i, b, s)
                o = values(i - 1, b, p, o)
            return softmax_parts(s) + (acc + out_proj(i - 1, o, l),)

        carry = lax.fori_loop(
            1, H - 1,
            lambda i, cr: step(i, cr, lambda i, b: start_step_unit(i, b + _LOOKAHEAD)),
            (p, l, jnp.zeros((B, D), _F32)),
        )

        def start_last(i, b):
            if b + _LOOKAHEAD < B:
                start_unit(i, i - 1, b + _LOOKAHEAD)
            else:
                start_unit(None, i, b + _LOOKAHEAD - B)

        p, l, acc = step(H - 1, carry, start_last)
        for b in range(_LOOKAHEAD, B):
            start_unit(None, H - 1, b)
        o = None
        for b in range(B):
            if b < len(f_chunks):
                start_rows(w1t_hbm, w1t_v, *f_chunks[b], s_w1.at[b])
            o = values(H - 1, b, p, o)
        start_rows(w2_hbm, w2_v, *f_chunks[0], s_w2.at[0])
        acc = acc + out_proj(H - 1, o, l)

        x1 = x + mod_b[:, :D] * acc
        h2 = (_layernorm(x1) * (1.0 + mod_c[:, :D]) + mod_b[:, D:]).astype(_BF16)
        for j in range(1, len(f_chunks)):
            start_rows(w2_hbm, w2_v, *f_chunks[j], s_w2.at[j])
        b1 = b1_v[...].astype(_F32).reshape(1, F)
        g = []
        for j, (f0, fn) in enumerate(f_chunks):
            _wait_filled(w1t_v.at[pl.ds(f0, fn)], s_w1.at[j])
            a = _dot_nt(h2, w1t_v[f0:f0 + fn, :]) + b1[:, f0:f0 + fn]
            g.append(jax.nn.gelu(a, approximate=True).astype(_BF16))
        y = b2_v[...].astype(_F32).reshape(1, D)
        for j, (f0, fn) in enumerate(f_chunks):
            _wait_filled(w2_v.at[pl.ds(f0, fn)], s_w2.at[j])
            y = y + _dot(g[j], w2_v[f0:f0 + fn, :])
        o_ref[...] = (x1 + mod_c[:, D:] * y).astype(o_ref.dtype)

    dma = pltpu.SemaphoreType.DMA
    out = pl.pallas_call(
        kernel,
        out_shape=jax.ShapeDtypeStruct((B, D), A_x.dtype),
        in_specs=[pl.BlockSpec(memory_space=pl.ANY)] * 11,
        scratch_shapes=[
            pltpu.VMEM((B, D), _BF16),
            pltpu.VMEM((B, D), _BF16),
            pltpu.VMEM((F,), _BF16),
            pltpu.VMEM((D,), _BF16),
            pltpu.VMEM((D, 6 * D), _BF16),
            pltpu.VMEM((D, H * _DH), _BF16),
            pltpu.VMEM((H * _DH, D), _BF16),
            pltpu.VMEM((F, D), _BF16),
            pltpu.VMEM((F, D), _BF16),
            pltpu.VMEM((n_slots, W, _DH), _BF16),
            pltpu.VMEM((n_slots, W, _DH), _BF16),
            pltpu.VMEM((H, B, _DH), _BF16),
            dma((4,)), dma((3,)), dma((n_qc,)), dma(()),
            dma((len(f_chunks),)), dma((len(f_chunks),)), dma((n_slots,)), dma((n_slots,)),
        ],
        compiler_params=pltpu.CompilerParams(vmem_limit_bytes=64 * 1024 * 1024),
    )(
        A_x.reshape(B, D), A_k_cache, A_v_cache, A_wq, A_wo,
        B_w1.T, B_b1, B_w2, B_b2, c, w_mod,
    )
    return out.reshape(B, Sq, D)
```

```python
import jax
import jax.numpy as jnp
from jax import lax
import jax.experimental.pallas as pl
import jax.experimental.pallas.tpu as pltpu

_BF16 = jnp.bfloat16
_F32 = jnp.float32
_HQ, _DH = 32, 128
_KV_ROWS = 80
_KV_CUTS = (0, 720, 1360)
_W_ROWS = 32
_LOOKAHEAD = 3


def _interleaved_pieces(total, cuts, size):
    ranges = list(zip(cuts, cuts[1:] + (total,)))
    pieces = []
    for off in range(0, max(hi - lo for lo, hi in ranges), size):
        for s, (lo, hi) in enumerate(ranges):
            if lo + off < hi:
                pieces.append((lo + off, min(size, hi - lo - off), s % 2))
    return pieces


def _layernorm(x, eps=1e-5):
    m = jnp.mean(x, axis=-1, keepdims=True)
    d = x - m
    v = jnp.mean(d * d, axis=-1, keepdims=True)
    return d * lax.rsqrt(v + eps)


def _dot(a, b):
    return jnp.dot(a, b, preferred_element_type=_F32)


def _dot_nt(a, b):
    return lax.dot_general(a, b, (((1,), (1,)), ((), ())), preferred_element_type=_F32)


def _wait_filled(ref, sem):
    pltpu.make_async_copy(ref, ref, sem).wait()


@jax.jit
def pallas_adaLN_cond__sliding_block_cached__dense_activation_gelu__decode_kernel(
    A_x: jax.Array,
    A_k_cache: jax.Array,
    A_v_cache: jax.Array,
    A_wq: jax.Array,
    A_wo: jax.Array,
    B_x: jax.Array,
    B_w1: jax.Array,
    B_b1: jax.Array,
    B_w2: jax.Array,
    B_b2: jax.Array,
    c: jax.Array,
    w_mod: jax.Array,
):
    del B_x
    B, Sq, D = A_x.shape
    Hkv, Sk = A_k_cache.shape[1], A_k_cache.shape[2]
    F = B_w1.shape[1]
    assert Sq == 1 and Hkv == _HQ
    W = min(4096, max(256, Sk // 4))
    S0 = Sk - W
    H = _HQ
    n_units = H * B
    n_slots = 2 * B
    assert _LOOKAHEAD < B
    kv_pieces = _interleaved_pieces(W, _KV_CUTS, _KV_ROWS)
    QC = 1024
    n_qc = H * _DH // QC
    f_chunks = [(0, 640), (640, 576), (1216, 512)]
    assert sum(n for _, n in f_chunks) == F

    def kernel(
        x_hbm, k_hbm, v_hbm, wq_hbm, wo_hbm, w1t_hbm, b1_hbm, w2_hbm, b2_hbm, c_hbm, wm_hbm,
        o_ref,
        x_v, c_v, b1_v, b2_v, wm_v, wq_v, wo_v, w1t_v, w2_v, k_v, v_v, q_v,
        s_small, s_wm, s_wq, s_wo, s_w1, s_w2, s_k, s_v,
    ):
        def start_cols(src, dst, col0, ncols, sem):
            def body(i, _):
                for p in range(2):
                    r = pl.ds(pl.multiple_of((2 * i + p) * 16, 16), 16)
                    pltpu.make_async_copy(
                        src.at[r, pl.ds(col0, ncols)], dst.at[r, pl.ds(col0, ncols)], sem
                    ).start(priority=p)
            lax.fori_loop(0, D // 32, body, None)

        def start_rows(src, dst, row0, nrows, sem):
            def body(i, _):
                for p in range(2):
                    r = pl.ds(pl.multiple_of(row0 + (2 * i + p) * _W_ROWS, _W_ROWS), _W_ROWS)
                    pltpu.make_async_copy(src.at[r], dst.at[r], sem).start(priority=p)
            lax.fori_loop(0, nrows // (2 * _W_ROWS), body, None)

        def kv_copy(src, dst, sem, h, b, r0, n):
            slot = (h % 2) * B + b
            return pltpu.make_async_copy(
                src.at[b, h, pl.ds(S0 + r0, n)], dst.at[slot, pl.ds(r0, n)], sem.at[slot]
            )

        def start_unit(hk, hv, b):
            for r0, n, p in kv_pieces:
                if hk is not None:
                    kv_copy(k_hbm, k_v, s_k, hk, b, r0, n).start(priority=p)
                if hv is not None:
                    kv_copy(v_hbm, v_v, s_v, hv, b, r0, n).start(priority=1 - p)

        def start_step_unit(i, b):
            i, b = i + b // B, b % B
            start_unit(i, i - 1, b)

        def wait_cols(dst, col0, ncols, sem):
            _wait_filled(dst.at[:, pl.ds(col0, ncols)], sem)

        def scores(h, b, s):
            slot = (h % 2) * B + b
            _wait_filled(k_v.at[slot], s_k.at[slot])
            sb = _dot_nt(q_v[h], k_v[slot])
            return sb if s is None else jnp.where(lax.broadcasted_iota(jnp.int32, sb.shape, 0) == b, sb, s)

        def values(h, b, p, o):
            slot = (h % 2) * B + b
            _wait_filled(v_v.at[slot], s_v.at[slot])
            ob = _dot(p, v_v[slot])
            return ob if o is None else jnp.where(lax.broadcasted_iota(jnp.int32, ob.shape, 0) == b, ob, o)

        def softmax_parts(s):
            s = s * (_DH ** -0.5)
            e = jnp.exp(s - jnp.max(s, axis=-1, keepdims=True))
            return e.astype(_BF16), jnp.sum(e, axis=-1, keepdims=True)

        def out_proj(h, o, l):
            r = pl.ds(pl.multiple_of(h * _DH, _DH), _DH)
            return _dot((o / l).astype(_BF16), wo_v[r, :])

        small = [
            pltpu.make_async_copy(src, dst, s_small.at[j])
            for j, (src, dst) in enumerate(
                ((c_hbm, c_v), (x_hbm, x_v), (b1_hbm, b1_v), (b2_hbm, b2_v))
            )
        ]
        for cp in small:
            cp.start()
        start_cols(wm_hbm, wm_v, 0, 2 * D, s_wm.at[0])
        start_cols(wq_hbm, wq_v, 0, QC, s_wq.at[0])
        start_cols(wq_hbm, wq_v, QC, QC, s_wq.at[1])
        for cp in small:
            cp.wait()
        cf = c_v[...].astype(_F32)
        sc = (cf * jax.nn.sigmoid(cf)).astype(_BF16)
        x = x_v[...].astype(_F32)
        wait_cols(wm_v, 0, 2 * D, s_wm.at[0])
        mod_a = _dot(sc, wm_v[:, 0:2 * D])
        h1 = (_layernorm(x) * (1.0 + mod_a[:, D:]) + mod_a[:, :D]).astype(_BF16)

        def q_chunk(j):
            wait_cols(wq_v, j * QC, QC, s_wq.at[j])
            q = _dot(h1, wq_v[:, j * QC:(j + 1) * QC]).astype(_BF16)
            for t in range(QC // _DH):
                q_v[j * (QC // _DH) + t] = q[:, t * _DH:(t + 1) * _DH]

        start_cols(wq_hbm, wq_v, 2 * QC, QC, s_wq.at[2])
        q_chunk(0)
        start_cols(wq_hbm, wq_v, 3 * QC, QC, s_wq.at[3])
        q_chunk(1)
        start_cols(wm_hbm, wm_v, 2 * D, 2 * D, s_wm.at[1])
        q_chunk(2)
        start_cols(wm_hbm, wm_v, 4 * D, 2 * D, s_wm.at[2])
        q_chunk(3)
        start_rows(wo_hbm, wo_v, 0, 1024, s_wo)
        wait_cols(wm_v, 2 * D, 2 * D, s_wm.at[1])
        mod_b = _dot(sc, wm_v[:, 2 * D:4 * D])
        start_rows(wo_hbm, wo_v, 1024, 1024, s_wo)
        wait_cols(wm_v, 4 * D, 2 * D, s_wm.at[2])
        mod_c = _dot(sc, wm_v[:, 4 * D:6 * D])
        start_rows(wo_hbm, wo_v, 2048, 2048, s_wo)

        for b in range(B):
            start_unit(0, None, b)
        s = None
        for b in range(B):
            if b >= B - _LOOKAHEAD - 1 + 1:
                start_unit(1, 0, b - (B - _LOOKAHEAD))
            s = scores(0, b, s)
        p, l = softmax_parts(s)
        _wait_filled(wo_v, s_wo)

        def step(i, carry, start):
            p, l, acc = carry
            s = o = None
            for b in range(B):
                start(i, b)
                s = scores(i, b, s)
                o = values(i - 1, b, p, o)
            return softmax_parts(s) + (acc + out_proj(i - 1, o, l),)

        carry = lax.fori_loop(
            1, H - 1,
            lambda i, cr: step(i, cr, lambda i, b: start_step_unit(i, b + _LOOKAHEAD)),
            (p, l, jnp.zeros((B, D), _F32)),
        )

        def start_last(i, b):
            if b + _LOOKAHEAD < B:
                start_unit(i, i - 1, b + _LOOKAHEAD)
            else:
                start_unit(None, i, b + _LOOKAHEAD - B)

        p, l, acc = step(H - 1, carry, start_last)
        for b in range(_LOOKAHEAD, B):
            start_unit(None, H - 1, b)
        o = None
        for b in range(B):
            if b < len(f_chunks):
                start_rows(w1t_hbm, w1t_v, *f_chunks[b], s_w1.at[b])
            o = values(H - 1, b, p, o)
        start_rows(w2_hbm, w2_v, *f_chunks[0], s_w2.at[0])
        acc = acc + out_proj(H - 1, o, l)

        x1 = x + mod_b[:, :D] * acc
        h2 = (_layernorm(x1) * (1.0 + mod_c[:, :D]) + mod_b[:, D:]).astype(_BF16)
        for j in range(1, len(f_chunks)):
            start_rows(w2_hbm, w2_v, *f_chunks[j], s_w2.at[j])
        b1 = b1_v[...].astype(_F32).reshape(1, F)
        g = []
        for j, (f0, fn) in enumerate(f_chunks):
            _wait_filled(w1t_v.at[pl.ds(f0, fn)], s_w1.at[j])
            a = _dot_nt(h2, w1t_v[f0:f0 + fn, :]) + b1[:, f0:f0 + fn]
            g.append(jax.nn.gelu(a, approximate=True).astype(_BF16))
        y = b2_v[...].astype(_F32).reshape(1, D)
        for j, (f0, fn) in enumerate(f_chunks):
            _wait_filled(w2_v.at[pl.ds(f0, fn)], s_w2.at[j])
            y = y + _dot(g[j], w2_v[f0:f0 + fn, :])
        o_ref[...] = (x1 + mod_c[:, D:] * y).astype(o_ref.dtype)

    dma = pltpu.SemaphoreType.DMA
    out = pl.pallas_call(
        kernel,
        out_shape=jax.ShapeDtypeStruct((B, D), A_x.dtype),
        in_specs=[pl.BlockSpec(memory_space=pl.ANY)] * 11,
        scratch_shapes=[
            pltpu.VMEM((B, D), _BF16),
            pltpu.VMEM((B, D), _BF16),
            pltpu.VMEM((F,), _BF16),
            pltpu.VMEM((D,), _BF16),
            pltpu.VMEM((D, 6 * D), _BF16),
            pltpu.VMEM((D, H * _DH), _BF16),
            pltpu.VMEM((H * _DH, D), _BF16),
            pltpu.VMEM((F, D), _BF16),
            pltpu.VMEM((F, D), _BF16),
            pltpu.VMEM((n_slots, W, _DH), _BF16),
            pltpu.VMEM((n_slots, W, _DH), _BF16),
            pltpu.VMEM((H, B, _DH), _BF16),
            dma((4,)), dma((3,)), dma((n_qc,)), dma(()),
            dma((len(f_chunks),)), dma((len(f_chunks),)), dma((n_slots,)), dma((n_slots,)),
        ],
        compiler_params=pltpu.CompilerParams(vmem_limit_bytes=64 * 1024 * 1024),
    )(
        A_x.reshape(B, D), A_k_cache, A_v_cache, A_wq, A_wo,
        B_w1.T, B_b1, B_w2, B_b2, c, w_mod,
    )
    return out.reshape(B, Sq, D)
```

```python
import jax
import jax.numpy as jnp
from jax import lax
import jax.experimental.pallas as pl
import jax.experimental.pallas.tpu as pltpu

_BF16 = jnp.bfloat16
_F32 = jnp.float32
_HQ, _DH = 32, 128
_KV_ROWS = 80
_KV_CUTS = (0, 720, 1360)
_LOOKAHEAD = 3


def _interleaved_pieces(total, cuts, size):
    ranges = list(zip(cuts, cuts[1:] + (total,)))
    pieces = []
    for off in range(0, max(hi - lo for lo, hi in ranges), size):
        for s, (lo, hi) in enumerate(ranges):
            if lo + off < hi:
                pieces.append((lo + off, min(size, hi - lo - off), s % 2))
    return pieces


def _layernorm(x, eps=1e-5):
    m = jnp.mean(x, axis=-1, keepdims=True)
    d = x - m
    v = jnp.mean(d * d, axis=-1, keepdims=True)
    return d * lax.rsqrt(v + eps)


def _dot(a, b):
    return jnp.dot(a, b, preferred_element_type=_F32)


def _dot_nt(a, b):
    return lax.dot_general(a, b, (((1,), (1,)), ((), ())), preferred_element_type=_F32)


def _wait_filled(ref, sem):
    pltpu.make_async_copy(ref, ref, sem).wait()


class _WeightStream:
    def __init__(self, src, dst, sem, row0, nrows, band, ncols):
        self.src, self.dst, self.sem = src, dst, sem
        self.row0, self.nrows, self.band, self.ncols = row0, nrows, band, ncols
        assert nrows % (2 * band) == 0
        self.half = nrows // (2 * band)
        self.steps = self.half // 3
        self.cuts = (0, self.steps, self.half - self.steps)

    def _copy_bands(self, i, thirds):
        for c0 in range(0, self.src.shape[1], self.ncols):
            for s in thirds:
                for side in range(2):
                    r0 = self.row0 + (self.cuts[s] + side * self.half + i) * self.band
                    idx = (pl.ds(pl.multiple_of(r0, self.band), self.band), pl.ds(c0, self.ncols))
                    pltpu.make_async_copy(self.src.at[idx], self.dst.at[idx], self.sem).start(
                        priority=(s + side) % 2
                    )

    def start(self, part=0, parts=1):
        lo, hi = lax.div(self.steps * part, parts), lax.div(self.steps * (part + 1), parts)
        lax.fori_loop(lo, hi, lambda i, _: self._copy_bands(i, (0, 1, 2)), None)
        if self.half > 3 * self.steps:

            @pl.when(jnp.int32(part) == parts - 1)
            def _():
                lax.fori_loop(
                    self.steps, self.half - 2 * self.steps,
                    lambda i, _: self._copy_bands(i, (1,)), None,
                )

    def wait(self):
        _wait_filled(self.dst.at[pl.ds(self.row0, self.nrows)], self.sem)


@jax.jit
def pallas_adaLN_cond__sliding_block_cached__dense_activation_gelu__decode_kernel(
    A_x: jax.Array,
    A_k_cache: jax.Array,
    A_v_cache: jax.Array,
    A_wq: jax.Array,
    A_wo: jax.Array,
    B_x: jax.Array,
    B_w1: jax.Array,
    B_b1: jax.Array,
    B_w2: jax.Array,
    B_b2: jax.Array,
    c: jax.Array,
    w_mod: jax.Array,
):
    del B_x
    B, Sq, D = A_x.shape
    Hkv, Sk = A_k_cache.shape[1], A_k_cache.shape[2]
    F = B_w1.shape[1]
    assert Sq == 1 and Hkv == _HQ and B == 4
    W = min(4096, max(256, Sk // 4))
    S0 = Sk - W
    H = _HQ
    n_units = H * B
    n_slots = _LOOKAHEAD + 1
    kv_pieces = _interleaved_pieces(W, _KV_CUTS, _KV_ROWS)
    QC = 512
    F0 = 1536

    def kernel(
        x_hbm, k_hbm, v_hbm, wq_hbm, wo_hbm, w1t_hbm, b1_hbm, w2_hbm, b2_hbm, c_hbm, wm_hbm,
        o_ref,
        x_v, c_v, b1_v, b2_v, wm_v, wq_v, wo_v, w1t_v, w2_v, k_v, v_v, q_v,
        mod_v, p_v, l_v, o_v, acc_v,
        s_small, s_w, s_k, s_v,
    ):
        wm = _WeightStream(wm_hbm, wm_v, s_w.at[0], 0, D, 8, 2 * D)
        wq = _WeightStream(wq_hbm, wq_v, s_w.at[1], 0, D, 8, 1024)
        wo = _WeightStream(wo_hbm, wo_v, s_w.at[2], 0, H * _DH, 16, D)
        w1 = _WeightStream(w1t_hbm, w1t_v, s_w.at[3], 0, F, 16, D)
        w2a = _WeightStream(w2_hbm, w2_v, s_w.at[4], 0, F0, 16, D)
        w2b = _WeightStream(w2_hbm, w2_v, s_w.at[5], F0, F - F0, 16, D)
        K, V = (k_hbm, k_v, s_k), (v_hbm, v_v, s_v)

        def window_copy(cache, u, r0, n):
            src, dst, sem = cache
            slot = lax.rem(u, n_slots)
            return pltpu.make_async_copy(
                src.at[lax.rem(u, B), lax.div(u, B), pl.ds(S0 + r0, n)],
                dst.at[slot, pl.ds(r0, n)],
                sem.at[slot],
            )

        def start_step(u):
            for r0, n, p in kv_pieces:
                window_copy(K, u, r0, n).start(priority=p)
                window_copy(V, u - 1, r0, n).start(priority=1 - p)

        def start_window(cache, u):
            for p in range(2):
                window_copy(cache, jnp.int32(u), p * W // 2, W // 2).start(priority=p)

        def wait_window(cache, u):
            _, dst, sem = cache
            slot = lax.rem(u, n_slots)
            _wait_filled(dst.at[slot], sem.at[slot])
            return dst[slot]

        small = [
            pltpu.make_async_copy(src, dst, s_small.at[j])
            for j, (src, dst) in enumerate(
                ((c_hbm, c_v), (x_hbm, x_v), (b1_hbm, b1_v), (b2_hbm, b2_v))
            )
        ]
        wm.start()
        for cp in small:
            cp.start()
        acc_v[...] = jnp.zeros(acc_v.shape, _F32)
        o_v[...] = jnp.zeros(o_v.shape, _F32)

        @pl.loop(0, 3)
        def _(j):
            wq.start(j, 3)

            @pl.when(j == 0)
            def _():
                for cp in small:
                    cp.wait()
                wm.wait()

            cf = c_v[...].astype(_F32)
            sc = (cf * jax.nn.sigmoid(cf)).astype(_BF16)

            @pl.loop(2 * j, 2 * j + 2)
            def _(t):
                mod_v[t] = _dot(sc, wm_v[:, pl.ds(pl.multiple_of(t * D, _DH), D)])

        x = x_v[...].astype(_F32)
        h1 = (_layernorm(x) * (1.0 + mod_v[1]) + mod_v[0]).astype(_BF16)
        n_qc = H * _DH // QC

        @pl.loop(0, 2)
        def _(j):
            wo.start(j, 2)

            @pl.when(j == 0)
            def _():
                wq.wait()

            @pl.loop(j * (n_qc // 2), (j + 1) * (n_qc // 2))
            def _(t):
                q = _dot(h1, wq_v[:, pl.ds(pl.multiple_of(t * QC, QC), QC)]).astype(_BF16)
                for i in range(QC // _DH):
                    q_v[t * (QC // _DH) + i] = q[:, i * _DH:(i + 1) * _DH]

        start_window(K, 0)

        @pl.loop(1 - _LOOKAHEAD, n_units + 1)
        def _(u):
            @pl.when(u + _LOOKAHEAD < n_units)
            def _():
                start_step(u + _LOOKAHEAD)

            @pl.when(u + _LOOKAHEAD == n_units)
            def _():
                start_window(V, n_units - 1)
                w1.start()

            @pl.when(u + _LOOKAHEAD == n_units + 1)
            def _():
                w2a.start()
                w2b.start()

            @pl.when(u == 0)
            def _():
                wo.wait()

            @pl.when(u > 0)
            def _():
                b = lax.rem(u - 1, B)
                o = _dot(p_v[...], wait_window(V, u - 1)) / l_v[...]
                o = jnp.where(lax.broadcasted_iota(jnp.int32, o.shape, 0) == b, o, o_v[...])
                o_v[...] = o

                @pl.when(b == B - 1)
                def _():
                    r = pl.ds(pl.multiple_of(lax.div(u - 1, B) * _DH, _DH), _DH)
                    acc_v[...] += _dot(o.astype(_BF16), wo_v[r, :])

            @pl.when(jnp.logical_and(u >= 0, u < n_units))
            def _():
                s = _dot_nt(q_v[lax.div(u, B)], wait_window(K, u)) * (_DH ** -0.5)
                e = jnp.exp(s - jnp.max(s, axis=-1, keepdims=True))
                p_v[...] = e.astype(_BF16)
                l_v[...] = jnp.broadcast_to(jnp.sum(e, axis=-1, keepdims=True), l_v.shape)

        x1 = x + mod_v[2] * acc_v[...]
        h2 = (_layernorm(x1) * (1.0 + mod_v[4]) + mod_v[3]).astype(_BF16)
        w1.wait()
        a = _dot_nt(h2, w1t_v[...]) + b1_v[...].astype(_F32).reshape(1, F)
        g = jax.nn.gelu(a, approximate=True).astype(_BF16)
        w2a.wait()
        y = b2_v[...].astype(_F32).reshape(1, D) + _dot(g[:, :F0], w2_v[:F0, :])
        w2b.wait()
        y = y + _dot(g[:, F0:], w2_v[F0:, :])
        o_ref[...] = (x1 + mod_v[5] * y).astype(o_ref.dtype)

    dma = pltpu.SemaphoreType.DMA
    out = pl.pallas_call(
        kernel,
        out_shape=jax.ShapeDtypeStruct((B, D), A_x.dtype),
        in_specs=[pl.BlockSpec(memory_space=pl.ANY)] * 11,
        scratch_shapes=[
            pltpu.VMEM((B, D), _BF16),
            pltpu.VMEM((B, D), _BF16),
            pltpu.VMEM((F,), _BF16),
            pltpu.VMEM((D,), _BF16),
            pltpu.VMEM((D, 6 * D), _BF16),
            pltpu.VMEM((D, H * _DH), _BF16),
            pltpu.VMEM((H * _DH, D), _BF16),
            pltpu.VMEM((F, D), _BF16),
            pltpu.VMEM((F, D), _BF16),
            pltpu.VMEM((n_slots, W, _DH), _BF16),
            pltpu.VMEM((n_slots, W, _DH), _BF16),
            pltpu.VMEM((H, B, _DH), _BF16),
            pltpu.VMEM((6, B, D), _F32),
            pltpu.VMEM((B, W), _BF16),
            pltpu.VMEM((B, _DH), _F32),
            pltpu.VMEM((B, _DH), _F32),
            pltpu.VMEM((B, D), _F32),
            dma((4,)), dma((6,)), dma((n_slots,)), dma((n_slots,)),
        ],
        compiler_params=pltpu.CompilerParams(vmem_limit_bytes=64 * 1024 * 1024),
    )(
        A_x.reshape(B, D), A_k_cache, A_v_cache, A_wq, A_wo,
        B_w1.T, B_b1, B_w2, B_b2, c, w_mod,
    )
    return out.reshape(B, Sq, D)
```

```python
import jax
import jax.numpy as jnp
from jax import lax
import jax.experimental.pallas as pl
import jax.experimental.pallas.tpu as pltpu

_BF16 = jnp.bfloat16
_F32 = jnp.float32
_HQ, _DH = 32, 128
_KV_ROWS = 80
_KV_CUTS = (0, 720, 1360)
_W2_CUTS = (0, 768, 1280, 1536)
_LOOKAHEAD = 3


def _interleaved_pieces(total, cuts, size):
    ranges = list(zip(cuts, cuts[1:] + (total,)))
    pieces = []
    for off in range(0, max(hi - lo for lo, hi in ranges), size):
        for s, (lo, hi) in enumerate(ranges):
            if lo + off < hi:
                pieces.append((lo + off, min(size, hi - lo - off), s % 2))
    return pieces


def _layernorm(x, eps=1e-5):
    m = jnp.mean(x, axis=-1, keepdims=True)
    d = x - m
    v = jnp.mean(d * d, axis=-1, keepdims=True)
    return d * lax.rsqrt(v + eps)


def _dot(a, b):
    return jnp.dot(a, b, preferred_element_type=_F32)


def _dot_nt(a, b):
    return lax.dot_general(a, b, (((1,), (1,)), ((), ())), preferred_element_type=_F32)


def _wait_filled(ref, sem):
    pltpu.make_async_copy(ref, ref, sem).wait()


class _WeightStream:
    def __init__(self, src, dst, sem, row0, nrows, band, ncols):
        self.src, self.dst, self.sem = src, dst, sem
        self.row0, self.nrows, self.band, self.ncols = row0, nrows, band, ncols
        assert nrows % (2 * band) == 0
        self.half = nrows // (2 * band)
        self.steps = self.half // 3
        self.cuts = (0, self.steps, self.half - self.steps)

    def _copy_bands(self, i, thirds):
        for c0 in range(0, self.src.shape[1], self.ncols):
            for s in thirds:
                for side in range(2):
                    r0 = self.row0 + (self.cuts[s] + side * self.half + i) * self.band
                    idx = (pl.ds(pl.multiple_of(r0, self.band), self.band), pl.ds(c0, self.ncols))
                    pltpu.make_async_copy(self.src.at[idx], self.dst.at[idx], self.sem).start(
                        priority=(s + side) % 2
                    )

    def start(self, part=0, parts=1):
        if self.steps:
            lo, hi = lax.div(self.steps * part, parts), lax.div(self.steps * (part + 1), parts)
            lax.fori_loop(lo, hi, lambda i, _: self._copy_bands(i, (0, 1, 2)), None)
        if self.half > 3 * self.steps:

            @pl.when(jnp.int32(part) == parts - 1)
            def _():
                lax.fori_loop(
                    self.steps, self.half - 2 * self.steps,
                    lambda i, _: self._copy_bands(i, (1,)), None,
                )

    def wait(self):
        _wait_filled(self.dst.at[pl.ds(self.row0, self.nrows)], self.sem)


@jax.jit
def pallas_adaLN_cond__sliding_block_cached__dense_activation_gelu__decode_kernel(
    A_x: jax.Array,
    A_k_cache: jax.Array,
    A_v_cache: jax.Array,
    A_wq: jax.Array,
    A_wo: jax.Array,
    B_x: jax.Array,
    B_w1: jax.Array,
    B_b1: jax.Array,
    B_w2: jax.Array,
    B_b2: jax.Array,
    c: jax.Array,
    w_mod: jax.Array,
):
    del B_x
    B, Sq, D = A_x.shape
    Hkv, Sk = A_k_cache.shape[1], A_k_cache.shape[2]
    F = B_w1.shape[1]
    assert Sq == 1 and Hkv == _HQ and B == 4
    W = min(4096, max(256, Sk // 4))
    S0 = Sk - W
    H = _HQ
    n_units = H * B
    n_slots = _LOOKAHEAD + 1
    kv_pieces = _interleaved_pieces(W, _KV_CUTS, _KV_ROWS)
    QC = 512
    w2_chunks = list(zip(_W2_CUTS, _W2_CUTS[1:] + (F,)))

    def kernel(
        x_hbm, k_hbm, v_hbm, wq_hbm, wo_hbm, w1t_hbm, b1_hbm, w2_hbm, b2_hbm, c_hbm, wm_hbm,
        o_ref,
        x_v, c_v, b1_v, b2_v, wm_v, wq_v, wo_v, w1t_v, w2_v, k_v, v_v, q_v,
        mod_v, p_v, l_v, o_v, acc_v,
        s_small, s_w, s_w2, s_k, s_v,
    ):
        wm = _WeightStream(wm_hbm, wm_v, s_w.at[0], 0, D, 8, 2 * D)
        wq = _WeightStream(wq_hbm, wq_v, s_w.at[1], 0, D, 8, 1024)
        wo = _WeightStream(wo_hbm, wo_v, s_w.at[2], 0, H * _DH, 16, D)
        w1 = _WeightStream(w1t_hbm, w1t_v, s_w.at[3], 0, F, 16, D)
        w2 = [
            _WeightStream(w2_hbm, w2_v, s_w2.at[j], lo, hi - lo, 16, D)
            for j, (lo, hi) in enumerate(w2_chunks)
        ]
        K, V = (k_hbm, k_v, s_k), (v_hbm, v_v, s_v)

        def slot_of(cache, u):
            slot = lax.rem(u, n_slots)
            return slot if cache is K else jnp.where(u == n_units - 1, n_slots, slot)

        def start_step(u):
            windows = ((K, u), (V, lax.rem(u + (n_units - 1), n_units)))
            for r0, n, p in kv_pieces:
                for side, (cache, w) in enumerate(windows):
                    src, dst, sem = cache
                    slot = slot_of(cache, w)
                    pltpu.make_async_copy(
                        src.at[lax.rem(w, B), lax.div(w, B), pl.ds(S0 + r0, n)],
                        dst.at[slot, pl.ds(r0, n)],
                        sem.at[slot],
                    ).start(priority=(p + side) % 2)

        def wait_window(cache, u):
            _, dst, sem = cache
            slot = slot_of(cache, u)
            _wait_filled(dst.at[slot], sem.at[slot])
            return dst[slot]

        small = [
            pltpu.make_async_copy(src, dst, s_small.at[j])
            for j, (src, dst) in enumerate(
                ((c_hbm, c_v), (x_hbm, x_v), (b1_hbm, b1_v), (b2_hbm, b2_v))
            )
        ]
        wm.start()
        for cp in small:
            cp.start()
        acc_v[...] = jnp.zeros(acc_v.shape, _F32)
        o_v[...] = jnp.zeros(o_v.shape, _F32)

        @pl.loop(0, 3)
        def _(j):
            wq.start(j, 3)

            @pl.when(j == 0)
            def _():
                for cp in small:
                    cp.wait()
                wm.wait()

            cf = c_v[...].astype(_F32)
            sc = (cf * jax.nn.sigmoid(cf)).astype(_BF16)

            @pl.loop(2 * j, 2 * j + 2)
            def _(t):
                mod_v[t] = _dot(sc, wm_v[:, pl.ds(pl.multiple_of(t * D, _DH), D)])

        x = x_v[...].astype(_F32)
        h1 = (_layernorm(x) * (1.0 + mod_v[1]) + mod_v[0]).astype(_BF16)
        n_qc = H * _DH // QC

        @pl.loop(0, 2)
        def _(j):
            wo.start(j, 2)

            @pl.when(j == 0)
            def _():
                wq.wait()

            @pl.loop(j * (n_qc // 2), (j + 1) * (n_qc // 2))
            def _(t):
                q = _dot(h1, wq_v[:, pl.ds(pl.multiple_of(t * QC, QC), QC)]).astype(_BF16)
                for i in range(QC // _DH):
                    q_v[t * (QC // _DH) + i] = q[:, i * _DH:(i + 1) * _DH]

        @pl.loop(-_LOOKAHEAD, n_units + 1)
        def _(u):
            @pl.when(u + _LOOKAHEAD < n_units)
            def _():
                start_step(u + _LOOKAHEAD)

            t = u + _LOOKAHEAD - n_units

            @pl.when(jnp.logical_and(t >= 0, t < 2))
            def _():
                w1.start(t, 2)

            @pl.when(t >= 2)
            def _():
                w2[0].start(t - 2, _LOOKAHEAD - 1)

            @pl.when(u == 0)
            def _():
                wo.wait()

            @pl.when(u > 0)
            def _():
                b = lax.rem(u - 1, B)
                o = _dot(p_v[...], wait_window(V, u - 1)) / l_v[...]
                o = jnp.where(lax.broadcasted_iota(jnp.int32, o.shape, 0) == b, o, o_v[...])
                o_v[...] = o

                @pl.when(b == B - 1)
                def _():
                    r = pl.ds(pl.multiple_of(lax.div(u - 1, B) * _DH, _DH), _DH)
                    acc_v[...] += _dot(o.astype(_BF16), wo_v[r, :])

            @pl.when(jnp.logical_and(u >= 0, u < n_units))
            def _():
                s = _dot_nt(q_v[lax.div(u, B)], wait_window(K, u)) * (_DH ** -0.5)
                e = jnp.exp(s - jnp.max(s, axis=-1, keepdims=True))
                p_v[...] = e.astype(_BF16)
                l_v[...] = jnp.broadcast_to(jnp.sum(e, axis=-1, keepdims=True), l_v.shape)

        for chunk in w2[1:]:
            chunk.start()
        x1 = x + mod_v[2] * acc_v[...]
        h2 = (_layernorm(x1) * (1.0 + mod_v[4]) + mod_v[3]).astype(_BF16)
        w1.wait()
        a = _dot_nt(h2, w1t_v[...]) + b1_v[...].astype(_F32).reshape(1, F)
        g = jax.nn.gelu(a, approximate=True).astype(_BF16)
        y = b2_v[...].astype(_F32).reshape(1, D)
        for chunk, (lo, hi) in zip(w2, w2_chunks):
            chunk.wait()
            y = y + _dot(g[:, lo:hi], w2_v[lo:hi, :])
        o_ref[...] = (x1 + mod_v[5] * y).astype(o_ref.dtype)

    dma = pltpu.SemaphoreType.DMA
    out = pl.pallas_call(
        kernel,
        out_shape=jax.ShapeDtypeStruct((B, D), A_x.dtype),
        in_specs=[pl.BlockSpec(memory_space=pl.ANY)] * 11,
        scratch_shapes=[
            pltpu.VMEM((B, D), _BF16),
            pltpu.VMEM((B, D), _BF16),
            pltpu.VMEM((F,), _BF16),
            pltpu.VMEM((D,), _BF16),
            pltpu.VMEM((D, 6 * D), _BF16),
            pltpu.VMEM((D, H * _DH), _BF16),
            pltpu.VMEM((H * _DH, D), _BF16),
            pltpu.VMEM((F, D), _BF16),
            pltpu.VMEM((F, D), _BF16),
            pltpu.VMEM((n_slots, W, _DH), _BF16),
            pltpu.VMEM((n_slots + 1, W, _DH), _BF16),
            pltpu.VMEM((H, B, _DH), _BF16),
            pltpu.VMEM((6, B, D), _F32),
            pltpu.VMEM((B, W), _BF16),
            pltpu.VMEM((B, _DH), _F32),
            pltpu.VMEM((B, _DH), _F32),
            pltpu.VMEM((B, D), _F32),
            dma((4,)), dma((4,)), dma((len(_W2_CUTS),)), dma((n_slots,)), dma((n_slots + 1,)),
        ],
        compiler_params=pltpu.CompilerParams(vmem_limit_bytes=64 * 1024 * 1024),
    )(
        A_x.reshape(B, D), A_k_cache, A_v_cache, A_wq, A_wo,
        B_w1.T, B_b1, B_w2, B_b2, c, w_mod,
    )
    return out.reshape(B, Sq, D)
```

```python
import jax
import jax.numpy as jnp
from jax import lax
import jax.experimental.pallas as pl
import jax.experimental.pallas.tpu as pltpu

_BF16 = jnp.bfloat16
_F32 = jnp.float32
_HQ, _DH = 32, 128
_KV_ROUNDS = 9
_KV_CUTS = (0, 576, 1504)
_W2_CUTS = (0, 768, 1280, 1536)
_LOOKAHEAD = 3


def _interleaved_pieces(total, cuts, rounds):
    pieces = []
    for i in range(rounds):
        for s, (lo, hi) in enumerate(zip(cuts, cuts[1:] + (total,))):
            a, b = (lo + 16 * ((hi - lo) // 16 * j // rounds) for j in (i, i + 1))
            pieces.append((a, b - a, s % 2))
    return pieces


def _layernorm(x, eps=1e-5):
    m = jnp.mean(x, axis=-1, keepdims=True)
    d = x - m
    v = jnp.mean(d * d, axis=-1, keepdims=True)
    return d * lax.rsqrt(v + eps)


def _dot(a, b):
    return jnp.dot(a, b, preferred_element_type=_F32)


def _dot_nt(a, b):
    return lax.dot_general(a, b, (((1,), (1,)), ((), ())), preferred_element_type=_F32)


def _wait_filled(ref, sem):
    pltpu.make_async_copy(ref, ref, sem).wait()


class _WeightStream:
    def __init__(self, src, dst, sem, row0, nrows, band, ncols):
        self.src, self.dst, self.sem = src, dst, sem
        self.row0, self.nrows, self.band, self.ncols = row0, nrows, band, ncols
        assert nrows % (2 * band) == 0
        self.half = nrows // (2 * band)
        self.steps = self.half // 3
        self.cuts = (0, self.steps, self.half - self.steps)

    def _copy_bands(self, i, thirds):
        for c0 in range(0, self.src.shape[1], self.ncols):
            for s in thirds:
                for side in range(2):
                    r0 = self.row0 + (self.cuts[s] + side * self.half + i) * self.band
                    idx = (pl.ds(pl.multiple_of(r0, self.band), self.band), pl.ds(c0, self.ncols))
                    pltpu.make_async_copy(self.src.at[idx], self.dst.at[idx], self.sem).start(
                        priority=(s + side) % 2
                    )

    def start(self, part=0, parts=1):
        if self.steps:
            lo, hi = lax.div(self.steps * part, parts), lax.div(self.steps * (part + 1), parts)
            lax.fori_loop(lo, hi, lambda i, _: self._copy_bands(i, (0, 1, 2)), None)
        if self.half > 3 * self.steps:

            @pl.when(jnp.int32(part) == parts - 1)
            def _():
                lax.fori_loop(
                    self.steps, self.half - 2 * self.steps,
                    lambda i, _: self._copy_bands(i, (1,)), None,
                )

    def wait(self):
        _wait_filled(self.dst.at[pl.ds(self.row0, self.nrows)], self.sem)


@jax.jit
def pallas_adaLN_cond__sliding_block_cached__dense_activation_gelu__decode_kernel(
    A_x: jax.Array,
    A_k_cache: jax.Array,
    A_v_cache: jax.Array,
    A_wq: jax.Array,
    A_wo: jax.Array,
    B_x: jax.Array,
    B_w1: jax.Array,
    B_b1: jax.Array,
    B_w2: jax.Array,
    B_b2: jax.Array,
    c: jax.Array,
    w_mod: jax.Array,
):
    del B_x
    B, Sq, D = A_x.shape
    Hkv, Sk = A_k_cache.shape[1], A_k_cache.shape[2]
    F = B_w1.shape[1]
    assert Sq == 1 and Hkv == _HQ and B == 4
    W = min(4096, max(256, Sk // 4))
    S0 = Sk - W
    H = _HQ
    n_units = H * B
    n_slots = _LOOKAHEAD + 1
    kv_pieces = _interleaved_pieces(W, _KV_CUTS, _KV_ROUNDS)
    QC = 512
    w2_chunks = list(zip(_W2_CUTS, _W2_CUTS[1:] + (F,)))

    def kernel(
        x_hbm, k_hbm, v_hbm, wq_hbm, wo_hbm, w1t_hbm, b1_hbm, w2_hbm, b2_hbm, c_hbm, wm_hbm,
        o_ref,
        x_v, c_v, b1_v, b2_v, wm_v, wq_v, wo_v, w1t_v, w2_v, k_v, v_v, q_v,
        mod_v, p_v, l_v, o_v, acc_v,
        s_small, s_w, s_w2, s_k, s_v,
    ):
        wm = _WeightStream(wm_hbm, wm_v, s_w.at[0], 0, D, 8, 2 * D)
        wq = _WeightStream(wq_hbm, wq_v, s_w.at[1], 0, D, 8, 1024)
        wo = _WeightStream(wo_hbm, wo_v, s_w.at[2], 0, H * _DH, 16, D)
        w1 = _WeightStream(w1t_hbm, w1t_v, s_w.at[3], 0, F, 16, D)
        w2 = [
            _WeightStream(w2_hbm, w2_v, s_w2.at[j], lo, hi - lo, 16, D)
            for j, (lo, hi) in enumerate(w2_chunks)
        ]
        K, V = (k_hbm, k_v, s_k), (v_hbm, v_v, s_v)

        def slot_of(cache, u):
            slot = lax.rem(u, n_slots)
            return slot if cache is K else jnp.where(u == n_units - 1, n_slots, slot)

        def start_step(u):
            windows = ((K, u), (V, lax.rem(u + (n_units - 1), n_units)))
            for r0, n, p in kv_pieces:
                for side, (cache, w) in enumerate(windows):
                    src, dst, sem = cache
                    slot = slot_of(cache, w)
                    pltpu.make_async_copy(
                        src.at[lax.rem(w, B), lax.div(w, B), pl.ds(S0 + r0, n)],
                        dst.at[slot, pl.ds(r0, n)],
                        sem.at[slot],
                    ).start(priority=(p + side) % 2)

        def wait_window(cache, u):
            _, dst, sem = cache
            slot = slot_of(cache, u)
            _wait_filled(dst.at[slot], sem.at[slot])
            return dst[slot]

        small = [
            pltpu.make_async_copy(src, dst, s_small.at[j])
            for j, (src, dst) in enumerate(
                ((c_hbm, c_v), (x_hbm, x_v), (b1_hbm, b1_v), (b2_hbm, b2_v))
            )
        ]
        wm.start()
        for cp in small:
            cp.start()
        acc_v[...] = jnp.zeros(acc_v.shape, _F32)
        o_v[...] = jnp.zeros(o_v.shape, _F32)

        @pl.loop(0, 3)
        def _(j):
            wq.start(j, 3)

            @pl.when(j == 0)
            def _():
                for cp in small:
                    cp.wait()
                wm.wait()

            cf = c_v[...].astype(_F32)
            sc = (cf * jax.nn.sigmoid(cf)).astype(_BF16)

            @pl.loop(2 * j, 2 * j + 2)
            def _(t):
                mod_v[t] = _dot(sc, wm_v[:, pl.ds(pl.multiple_of(t * D, _DH), D)])

        x = x_v[...].astype(_F32)
        h1 = (_layernorm(x) * (1.0 + mod_v[1]) + mod_v[0]).astype(_BF16)
        n_qc = H * _DH // QC

        @pl.loop(0, 2)
        def _(j):
            wo.start(j, 2)

            @pl.when(j == 0)
            def _():
                wq.wait()

            @pl.loop(j * (n_qc // 2), (j + 1) * (n_qc // 2))
            def _(t):
                q = _dot(h1, wq_v[:, pl.ds(pl.multiple_of(t * QC, QC), QC)]).astype(_BF16)
                for i in range(QC // _DH):
                    q_v[t * (QC // _DH) + i] = q[:, i * _DH:(i + 1) * _DH]

        @pl.loop(-_LOOKAHEAD, n_units + 1)
        def _(u):
            @pl.when(u + _LOOKAHEAD < n_units)
            def _():
                start_step(u + _LOOKAHEAD)

            t = u + _LOOKAHEAD - n_units

            @pl.when(jnp.logical_and(t >= 0, t < 2))
            def _():
                w1.start(t, 2)

            @pl.when(t >= 2)
            def _():
                w2[0].start(t - 2, _LOOKAHEAD - 1)

            @pl.when(u == 0)
            def _():
                wo.wait()

            @pl.when(u > 0)
            def _():
                b = lax.rem(u - 1, B)
                o = _dot(p_v[...], wait_window(V, u - 1)) / l_v[...]
                o = jnp.where(lax.broadcasted_iota(jnp.int32, o.shape, 0) == b, o, o_v[...])
                o_v[...] = o

                @pl.when(b == B - 1)
                def _():
                    r = pl.ds(pl.multiple_of(lax.div(u - 1, B) * _DH, _DH), _DH)
                    acc_v[...] += _dot(o.astype(_BF16), wo_v[r, :])

            @pl.when(jnp.logical_and(u >= 0, u < n_units))
            def _():
                s = _dot_nt(q_v[lax.div(u, B)], wait_window(K, u)) * (_DH ** -0.5)
                e = jnp.exp(s - jnp.max(s, axis=-1, keepdims=True))
                p_v[...] = e.astype(_BF16)
                l_v[...] = jnp.broadcast_to(jnp.sum(e, axis=-1, keepdims=True), l_v.shape)

        for chunk in w2[1:]:
            chunk.start()
        x1 = x + mod_v[2] * acc_v[...]
        h2 = (_layernorm(x1) * (1.0 + mod_v[4]) + mod_v[3]).astype(_BF16)
        w1.wait()
        a = _dot_nt(h2, w1t_v[...]) + b1_v[...].astype(_F32).reshape(1, F)
        g = jax.nn.gelu(a, approximate=True).astype(_BF16)
        y = b2_v[...].astype(_F32).reshape(1, D)
        for chunk, (lo, hi) in zip(w2, w2_chunks):
            chunk.wait()
            y = y + _dot(g[:, lo:hi], w2_v[lo:hi, :])
        o_ref[...] = (x1 + mod_v[5] * y).astype(o_ref.dtype)

    dma = pltpu.SemaphoreType.DMA
    out = pl.pallas_call(
        kernel,
        out_shape=jax.ShapeDtypeStruct((B, D), A_x.dtype),
        in_specs=[pl.BlockSpec(memory_space=pl.ANY)] * 11,
        scratch_shapes=[
            pltpu.VMEM((B, D), _BF16),
            pltpu.VMEM((B, D), _BF16),
            pltpu.VMEM((F,), _BF16),
            pltpu.VMEM((D,), _BF16),
            pltpu.VMEM((D, 6 * D), _BF16),
            pltpu.VMEM((D, H * _DH), _BF16),
            pltpu.VMEM((H * _DH, D), _BF16),
            pltpu.VMEM((F, D), _BF16),
            pltpu.VMEM((F, D), _BF16),
            pltpu.VMEM((n_slots, W, _DH), _BF16),
            pltpu.VMEM((n_slots + 1, W, _DH), _BF16),
            pltpu.VMEM((H, B, _DH), _BF16),
            pltpu.VMEM((6, B, D), _F32),
            pltpu.VMEM((B, W), _BF16),
            pltpu.VMEM((B, _DH), _F32),
            pltpu.VMEM((B, _DH), _F32),
            pltpu.VMEM((B, D), _F32),
            dma((4,)), dma((4,)), dma((len(_W2_CUTS),)), dma((n_slots,)), dma((n_slots + 1,)),
        ],
        compiler_params=pltpu.CompilerParams(vmem_limit_bytes=64 * 1024 * 1024),
    )(
        A_x.reshape(B, D), A_k_cache, A_v_cache, A_wq, A_wo,
        B_w1.T, B_b1, B_w2, B_b2, c, w_mod,
    )
    return out.reshape(B, Sq, D)
```

```python
import jax
import jax.numpy as jnp
from jax import lax
import jax.experimental.pallas as pl
import jax.experimental.pallas.tpu as pltpu

_BF16 = jnp.bfloat16
_F32 = jnp.float32
_HQ, _DH = 32, 128
_KV_ROUNDS = 6
_KV_CUTS = (0, 576, 1344)
_W2_CUTS = (0, 768, 1280, 1536)
_LOOKAHEAD = 3


def _interleaved_pieces(total, cuts, rounds):
    pieces = []
    for i in range(rounds):
        for s, (lo, hi) in enumerate(zip(cuts, cuts[1:] + (total,))):
            a, b = (lo + 16 * ((hi - lo) // 16 * j // rounds) for j in (i, i + 1))
            pieces.append((a, b - a, s % 2))
    return pieces


def _layernorm(x, eps=1e-5):
    m = jnp.mean(x, axis=-1, keepdims=True)
    d = x - m
    v = jnp.mean(d * d, axis=-1, keepdims=True)
    return d * lax.rsqrt(v + eps)


def _dot(a, b):
    return jnp.dot(a, b, preferred_element_type=_F32)


def _dot_nt(a, b):
    return lax.dot_general(a, b, (((1,), (1,)), ((), ())), preferred_element_type=_F32)


def _wait_filled(ref, sem):
    pltpu.make_async_copy(ref, ref, sem).wait()


class _WeightStream:
    def __init__(self, src, dst, sem, row0, nrows, band, ncols):
        self.src, self.dst, self.sem = src, dst, sem
        self.row0, self.nrows, self.band, self.ncols = row0, nrows, band, ncols
        assert nrows % (2 * band) == 0
        self.half = nrows // (2 * band)
        self.steps = self.half // 3
        self.cuts = (0, self.steps, self.half - self.steps)

    def _copy_bands(self, i, thirds):
        for c0 in range(0, self.src.shape[1], self.ncols):
            for s in thirds:
                for side in range(2):
                    r0 = self.row0 + (self.cuts[s] + side * self.half + i) * self.band
                    idx = (pl.ds(pl.multiple_of(r0, self.band), self.band), pl.ds(c0, self.ncols))
                    pltpu.make_async_copy(self.src.at[idx], self.dst.at[idx], self.sem).start(
                        priority=(s + side) % 2
                    )

    def start(self, part=0, parts=1):
        if self.steps:
            lo, hi = lax.div(self.steps * part, parts), lax.div(self.steps * (part + 1), parts)
            lax.fori_loop(lo, hi, lambda i, _: self._copy_bands(i, (0, 1, 2)), None)
        if self.half > 3 * self.steps:

            @pl.when(jnp.int32(part) == parts - 1)
            def _():
                lax.fori_loop(
                    self.steps, self.half - 2 * self.steps,
                    lambda i, _: self._copy_bands(i, (1,)), None,
                )

    def wait(self):
        _wait_filled(self.dst.at[pl.ds(self.row0, self.nrows)], self.sem)


@jax.jit
def pallas_adaLN_cond__sliding_block_cached__dense_activation_gelu__decode_kernel(
    A_x: jax.Array,
    A_k_cache: jax.Array,
    A_v_cache: jax.Array,
    A_wq: jax.Array,
    A_wo: jax.Array,
    B_x: jax.Array,
    B_w1: jax.Array,
    B_b1: jax.Array,
    B_w2: jax.Array,
    B_b2: jax.Array,
    c: jax.Array,
    w_mod: jax.Array,
):
    del B_x
    B, Sq, D = A_x.shape
    Hkv, Sk = A_k_cache.shape[1], A_k_cache.shape[2]
    F = B_w1.shape[1]
    assert Sq == 1 and Hkv == _HQ and B == 4
    W = min(4096, max(256, Sk // 4))
    S0 = Sk - W
    H = _HQ
    n_steps = H * B
    n_slots = _LOOKAHEAD + 1
    kv_pieces = _interleaved_pieces(W, _KV_CUTS, _KV_ROUNDS)
    QC = 512
    w2_chunks = list(zip(_W2_CUTS, _W2_CUTS[1:] + (F,)))

    def kernel(
        x_hbm, k_hbm, v_hbm, wq_hbm, wo_hbm, w1t_hbm, b1_hbm, w2_hbm, b2_hbm, c_hbm, wm_hbm,
        o_ref,
        x_v, c_v, b1_v, b2_v, wm_v, wq_v, wo_v, w1t_v, w2_v, kv_v, q_v,
        mod_v, p_v, l_v, o_v, acc_v,
        s_small, s_w, s_w2, s_kv,
    ):
        wm = _WeightStream(wm_hbm, wm_v, s_w.at[0], 0, D, 8, 2 * D)
        wq = _WeightStream(wq_hbm, wq_v, s_w.at[1], 0, D, 8, 1024)
        wo = _WeightStream(wo_hbm, wo_v, s_w.at[2], 0, H * _DH, 16, D)
        w1 = _WeightStream(w1t_hbm, w1t_v, s_w.at[3], 0, F, 16, D)
        w2 = [
            _WeightStream(w2_hbm, w2_v, s_w2.at[j], lo, hi - lo, 16, D)
            for j, (lo, hi) in enumerate(w2_chunks)
        ]

        def head_and_batch(u):
            g = lax.div(u, 2)
            return 2 * lax.div(g, B), lax.rem(g, B)

        def start_windows(src, u):
            h, b = head_and_batch(u)
            slot = lax.rem(u, n_slots)
            for r0, n, p in kv_pieces:
                for j in range(2):
                    pltpu.make_async_copy(
                        src.at[b, h + j, pl.ds(S0 + r0, n)],
                        kv_v.at[slot, j, pl.ds(r0, n)],
                        s_kv.at[slot],
                    ).start(priority=(p + j) % 2)

        small = [
            pltpu.make_async_copy(src, dst, s_small.at[j])
            for j, (src, dst) in enumerate(
                ((c_hbm, c_v), (x_hbm, x_v), (b1_hbm, b1_v), (b2_hbm, b2_v))
            )
        ]
        wm.start()
        for cp in small:
            cp.start()
        acc_v[...] = jnp.zeros(acc_v.shape, _F32)
        o_v[...] = jnp.zeros(o_v.shape, _F32)

        @pl.loop(0, 3)
        def _(j):
            wq.start(j, 3)

            @pl.when(j == 0)
            def _():
                for cp in small:
                    cp.wait()
                wm.wait()

            cf = c_v[...].astype(_F32)
            sc = (cf * jax.nn.sigmoid(cf)).astype(_BF16)

            @pl.loop(2 * j, 2 * j + 2)
            def _(t):
                mod_v[t] = _dot(sc, wm_v[:, pl.ds(pl.multiple_of(t * D, _DH), D)])

        x = x_v[...].astype(_F32)
        h1 = (_layernorm(x) * (1.0 + mod_v[1]) + mod_v[0]).astype(_BF16)
        n_qc = H * _DH // QC

        @pl.loop(0, 2)
        def _(j):
            wo.start(j, 2)

            @pl.when(j == 0)
            def _():
                wq.wait()

            @pl.loop(j * (n_qc // 2), (j + 1) * (n_qc // 2))
            def _(t):
                q = _dot(h1, wq_v[:, pl.ds(pl.multiple_of(t * QC, QC), QC)]).astype(_BF16)
                for i in range(QC // _DH):
                    q_v[t * (QC // _DH) + i] = q[:, i * _DH:(i + 1) * _DH]

        @pl.loop(-_LOOKAHEAD, n_steps)
        def _(u):
            ahead = u + _LOOKAHEAD
            for parity, src in enumerate((k_hbm, v_hbm)):
                pl.when(jnp.logical_and(ahead < n_steps, lax.rem(ahead, 2) == parity))(
                    lambda src=src: start_windows(src, ahead)
                )

            t = ahead - n_steps

            @pl.when(jnp.logical_and(t >= 0, t < 2))
            def _():
                w1.start(t, 2)

            @pl.when(t == 2)
            def _():
                w2[0].start()

            @pl.when(u == 0)
            def _():
                wo.wait()

            @pl.when(u >= 0)
            def _():
                h, b = head_and_batch(u)
                slot = lax.rem(u, n_slots)
                _wait_filled(kv_v.at[slot], s_kv.at[slot])

                @pl.when(lax.rem(u, 2) == 0)
                def _():
                    @pl.loop(0, 2)
                    def _(j):
                        s = _dot_nt(q_v[h + j], kv_v[slot, j]) * (_DH ** -0.5)
                        e = jnp.exp(s - jnp.max(s, axis=-1, keepdims=True))
                        p_v[j] = e.astype(_BF16)
                        l_v[j] = jnp.broadcast_to(jnp.sum(e, axis=-1, keepdims=True), (B, _DH))

                @pl.when(lax.rem(u, 2) == 1)
                def _():
                    @pl.loop(0, 2)
                    def _(j):
                        o = _dot(p_v[j], kv_v[slot, j]) / l_v[j]
                        o = jnp.where(lax.broadcasted_iota(jnp.int32, o.shape, 0) == b, o, o_v[j])
                        o_v[j] = o

                        @pl.when(b == B - 1)
                        def _():
                            r = pl.ds(pl.multiple_of((h + j) * _DH, _DH), _DH)
                            acc_v[...] += _dot(o.astype(_BF16), wo_v[r, :])

        for chunk in w2[1:]:
            chunk.start()
        x1 = x + mod_v[2] * acc_v[...]
        h2 = (_layernorm(x1) * (1.0 + mod_v[4]) + mod_v[3]).astype(_BF16)
        w1.wait()
        a = _dot_nt(h2, w1t_v[...]) + b1_v[...].astype(_F32).reshape(1, F)
        g = jax.nn.gelu(a, approximate=True).astype(_BF16)
        y = b2_v[...].astype(_F32).reshape(1, D)
        for chunk, (lo, hi) in zip(w2, w2_chunks):
            chunk.wait()
            y = y + _dot(g[:, lo:hi], w2_v[lo:hi, :])
        o_ref[...] = (x1 + mod_v[5] * y).astype(o_ref.dtype)

    dma = pltpu.SemaphoreType.DMA
    out = pl.pallas_call(
        kernel,
        out_shape=jax.ShapeDtypeStruct((B, D), A_x.dtype),
        in_specs=[pl.BlockSpec(memory_space=pl.ANY)] * 11,
        scratch_shapes=[
            pltpu.VMEM((B, D), _BF16),
            pltpu.VMEM((B, D), _BF16),
            pltpu.VMEM((F,), _BF16),
            pltpu.VMEM((D,), _BF16),
            pltpu.VMEM((D, 6 * D), _BF16),
            pltpu.VMEM((D, H * _DH), _BF16),
            pltpu.VMEM((H * _DH, D), _BF16),
            pltpu.VMEM((F, D), _BF16),
            pltpu.VMEM((F, D), _BF16),
            pltpu.VMEM((n_slots, 2, W, _DH), _BF16),
            pltpu.VMEM((H, B, _DH), _BF16),
            pltpu.VMEM((6, B, D), _F32),
            pltpu.VMEM((2, B, W), _BF16),
            pltpu.VMEM((2, B, _DH), _F32),
            pltpu.VMEM((2, B, _DH), _F32),
            pltpu.VMEM((B, D), _F32),
            dma((4,)), dma((4,)), dma((len(_W2_CUTS),)), dma((n_slots,)),
        ],
        compiler_params=pltpu.CompilerParams(
            vmem_limit_bytes=64 * 1024 * 1024,
        ),
    )(
        A_x.reshape(B, D), A_k_cache, A_v_cache, A_wq, A_wo,
        B_w1.T, B_b1, B_w2, B_b2, c, w_mod,
    )
    return out.reshape(B, Sq, D)
```
